```python
import os as _os
_os.environ.setdefault("JAX_PLATFORMS", "cpu")
import jax
import jax.numpy as jnp

def _softmax(x, axis=-1):
    return jax.nn.softmax(x, axis=axis)
def _gelu(x):
    return jax.nn.gelu(x, approximate=True)
def _silu(x):
    return jax.nn.silu(x)
def _sigmoid(x):
    return jax.nn.sigmoid(x)
def _layernorm(x, axis=-1, eps=1e-5):
    m = jnp.mean(x, axis=axis, keepdims=True)
    v = jnp.var(x, axis=axis, keepdims=True)
    return (x - m) / jnp.sqrt(v + eps)
def _scatter_add(tgt, idx, src, axis=0):
    return tgt.at[idx].add(src)
def _segment_sum(src, seg, n):
    return jax.ops.segment_sum(src, seg, n)
class _Rng:
    def __init__(self, key):
        self._k = key
    def _next(self):
        self._k, sub = jax.random.split(self._k)
        return sub
    def normal(self, shape):
        return jax.random.normal(self._next(), shape, dtype=jnp.bfloat16)
    def randint(self, lo, hi, shape):
        return jax.random.randint(self._next(), shape, lo, hi, dtype=jnp.int32)
    def uniform(self, shape, lo=0.0, hi=1.0):
        return jax.random.uniform(self._next(), shape, jnp.bfloat16, lo, hi)
    def permutation(self, n):
        return jax.random.permutation(self._next(), n)


kernel_name = 'concat_heads__sliding_local_dilated__compressed_kv_cla__prompt'

def setup_inputs():
    _rng = _Rng(jax.random.key(int.from_bytes(__import__("os").urandom(4), "little")))
    _w = (lambda a: (lambda t: t.astype(jnp.bfloat16) if jnp.issubdtype(t.dtype, jnp.floating) else t)(jnp.asarray(a)))
    def _A_setup():
        B, S, D = 1, 2048, 640
        return {
            "x": _w((lambda *s: _rng.normal(s) * 0.2)(B, S, D)),
            "wqkv": _w((lambda *s: _rng.normal(s) * 0.2)(D, 3 * D)),
            "wo": _w((lambda *s: _rng.normal(s) * 0.05)(D, D)),
        }
    _A_in = _A_setup()

    def _B_setup():
        B, H, Sq, Sk, D, M = 1, 32, 2048, 2048, 128, 640
        Dc = 4 * D
        return {
            "x": _w((lambda *s: _rng.normal(s) * 0.8)(B, Sq, M)),
            "c_kv": _w((lambda *s: _rng.normal(s) * 0.8)(B, Sk, Dc)),
            "w_q": _w((lambda *s: _rng.normal(s) * 1.6)(M, H, D) * (M ** -0.5)),
            "w_uk": _w((lambda *s: _rng.normal(s) * 1.6)(Dc, H, D) * (Dc ** -0.5)),
            "w_uv": _w((lambda *s: _rng.normal(s) * 0.8)(Dc, H, D) * (Dc ** -0.5)),
            "w_o": _w((lambda *s: _rng.normal(s) * 0.8)(H, D, M) * ((H * D) ** -0.5)),
        }
    _B_in = _B_setup()

    return {
        "A_x": _A_in["x"],
        "A_wqkv": _A_in["wqkv"],
        "A_wo": _A_in["wo"],
        "B_x": _B_in["x"],
        "B_c_kv": _B_in["c_kv"],
        "B_w_q": _B_in["w_q"],
        "B_w_uk": _B_in["w_uk"],
        "B_w_uv": _B_in["w_uv"],
        "B_w_o": _B_in["w_o"],
    }

def reference(A_x, A_wqkv, A_wo, B_x, B_c_kv, B_w_q, B_w_uk, B_w_uv, B_w_o):
    def _A_ref(x, wqkv, wo):
        B, S, D = x.shape
        H = 32; Dh = D // H
        W, dil = 8, 2
        qkv = (lambda x, *d: x.transpose(*d))((x @ wqkv).reshape(B, S, 3, H, Dh), 2, 0, 3, 1, 4)
        q, k, v = qkv[0], qkv[1], qkv[2]
        scale = Dh ** -0.5
        pos = jnp.arange(S)
        off = jnp.arange(W) * dil
        idx = pos[:, None] - off[None, :]
        mask = idx >= 0
        idx_c = jnp.where(mask, idx, 0).reshape(-1)
        kg = k[:, :, idx_c, :].reshape(B, H, S, W, Dh)
        vg = v[:, :, idx_c, :].reshape(B, H, S, W, Dh)
        logits = jnp.einsum("bhsd,bhswd->bhsw", q, kg) * scale
        logits = jnp.where(mask[None, None, :, :], logits, -1e9)
        attn = _softmax(logits, axis=-1)
        o = jnp.einsum("bhsw,bhswd->bhsd", attn, vg)
        return (lambda x, *d: x.transpose(*d))(o, 0, 2, 1, 3).reshape(B, S, D) @ wo

    def _B_ref(x, c_kv, w_q, w_uk, w_uv, w_o):
        B, Sq, M = x.shape[0], x.shape[1], x.shape[2]
        Sk = c_kv.shape[1]
        H, D = w_q.shape[1], w_q.shape[2]
        q = jnp.einsum("bqm,mhd->bhqd", x, w_q)
        k = jnp.einsum("bkc,chd->bhkd", c_kv, w_uk)
        v = jnp.einsum("bkc,chd->bhkd", c_kv, w_uv)
        scores = jnp.einsum("bhqd,bhkd->bhqk", q, k) * (D ** -0.5)
        off = Sk - Sq
        qi = jnp.arange(Sq)[:, None]
        kj = jnp.arange(Sk)[None, :]
        cmask = kj <= (qi + off)
        scores = jnp.where(cmask[None, None], scores, -1e9)
        p = _softmax(scores, axis=-1)
        ctx = jnp.einsum("bhqk,bhkd->bhqd", p, v)
        return jnp.einsum("bhqd,hdm->bqm", ctx, w_o)

    a = _A_ref(A_x, A_wqkv, A_wo)
    b = _B_ref(B_x, B_c_kv, B_w_q, B_w_uk, B_w_uv, B_w_o)
    return jnp.concatenate([a, b], axis=-1)
```

```python
import numpy as np
import jax
import jax.numpy as jnp
from jax import lax
import jax.experimental.pallas as pl
import jax.experimental.pallas.tpu as pltpu

S, DM, DC, H, D = 2048, 640, 512, 32, 128
HA, DA, WIN, DIL = 32, 20, 8, 2
PAD = 16
NG = DM // 128
BQ = 256
RC = 512
RP = 256
RA = 32
NPAIR = H // 2
F32, BF16 = jnp.float32, jnp.bfloat16
LOG2E = 1.4426950408889634
NEG = -1e9 * LOG2E
NT = (((1,), (1,)), ((), ()))


def _dot(a, b):
    return jnp.dot(a, b, preferred_element_type=F32)


def _dot_nt(a, b):
    return lax.dot_general(a, b, NT, preferred_element_type=F32)


def _reduce(op, xs, group):
    def tree(ys):
        return ys[0] if len(ys) == 1 else op(tree(ys[:len(ys) // 2]), tree(ys[len(ys) // 2:]))
    r = xs[0]
    for n in range(1, len(xs), group):
        r = op(r, tree(xs[n:n + group]))
    return r


def _kernel(ax_h, wqkv_h, awo_h, bx_h, c_h, wq_h, wuk_h, wuv_h, wo_h, out_h,
            ax, wqkv, awo, bx, c, wq, wuk, wuv, wo, outa, outb,
            qkv, tmp, qs, ks, vs, ctx, acc, wq2, wkv,
            sem_w, sem_x, sem_b, sem_oa, sem_ob):
    def rows_of(i, n):
        return pl.ds(pl.multiple_of(i * n, n), n)

    def cp_wqkv(t):
        return pltpu.make_async_copy(
            wqkv_h.at[:, pl.ds(pl.multiple_of(t * DM, 128), DM)], wqkv.at[t], sem_w.at[t])

    def cp_ax(i):
        return pltpu.make_async_copy(ax_h.at[rows_of(i, RP)], ax.at[rows_of(i, RP)], sem_x.at[i])

    def cp_outa(i):
        return pltpu.make_async_copy(outa.at[rows_of(i, RP)], out_h.at[rows_of(i, RP), 0:DM], sem_oa.at[i])

    first = [(awo_h, awo), (wq_h, wq), (wuk_h, wuk), (wuv_h, wuv)]
    second = [(bx_h, bx), (c_h, c), (wo_h, wo)]
    cps = [pltpu.make_async_copy(s, d, sem_b.at[n]) for n, (s, d) in enumerate(first + second)]
    cps1, cps2 = cps[:len(first)], cps[len(first):]
    for t in range(3):
        cp_wqkv(t).start()
    for i in range(S // RP):
        cp_ax(i).start()

    def permute_rows(w):
        for g in range(NG):
            tmp[g] = w[:, g * 128:(g + 1) * 128]
        return jnp.concatenate(
            [jnp.concatenate([tmp[g, pl.ds(d, HA, stride=DA), :] for d in range(DA)], axis=0).astype(BF16)
             for g in range(NG)], axis=1)

    def a_wprep(t, _):
        cp_wqkv(t).wait()

        @pl.when(t == 0)
        def _():
            for cp in cps1:
                cp.start()

        wqkv[t] = permute_rows(wqkv[t].astype(F32).T)

    lax.fori_loop(0, 3, a_wprep, None)
    qkv[:, :, 0:PAD, :] = jnp.zeros((3, NG, PAD, 128), F32)
    acc[...] = jnp.zeros(acc.shape, F32)

    def a_proj(i, _):
        @pl.when(i == 1)
        def _():
            for cp in cps2:
                cp.start()

        cp_ax(i).wait()
        for t in range(3):
            y = _dot_nt(ax[rows_of(i, RP), :], wqkv[t])
            if t == 0:
                y = y * (DA ** -0.5 * LOG2E)
            for g in range(NG):
                qkv[t, g, pl.ds(pl.multiple_of(PAD + i * RP, PAD), RP), :] = y[:, g * 128:(g + 1) * 128]

    lax.fori_loop(0, S // RP, a_proj, None)
    for cp in cps1:
        cp.wait()
    awo[...] = permute_rows(awo[...].astype(F32))

    def a_attn(i):
        r0 = pl.multiple_of(i * RA, RA)
        q = qkv[0, :, pl.ds(r0 + PAD, RA), :]
        row = lax.broadcasted_iota(jnp.int32, (RA, 128), 0)
        logits = []
        for w in range(WIN):
            p = q * qkv[1, :, pl.ds(r0 + PAD - DIL * w, RA), :]
            s = p[0] + p[1] + p[2] + p[3] + p[4]
            s = s + pltpu.roll(s, 64, 1)
            s = s + pltpu.roll(s, 32, 1)
            if w > 0:
                s = jnp.where(row >= DIL * w - r0, s, NEG)
            logits.append(s)
        m = _reduce(jnp.maximum, logits, 1)
        es = [jnp.exp2(s - m) for s in logits]
        o = _reduce(jnp.add, [es[w][None] * qkv[2, :, pl.ds(r0 + PAD - DIL * w, RA), :] for w in range(WIN)], 1)
        o = o * (1.0 / _reduce(jnp.add, es, 1))[None]
        for g in range(NG):
            ax[pl.ds(r0, RA), g * 128:(g + 1) * 128] = o[g].astype(BF16)

    def prep(g, t):
        for dst, srcs in ((wq2, (wq,)), (wkv, (wuk, wuv))):
            n4 = srcs[0].shape[0] // H // 4
            for n, w in enumerate(srcs):
                base = pl.multiple_of(t * (n4 * NPAIR) + g * 4, 4)
                view = w.bitcast(jnp.uint32).at[pl.ds(base, (n4 - 1) * NPAIR + 4), :]
                rr = pl.ds(pl.multiple_of(t * n4, 16), n4)
                for r in range(4):
                    u = view[pl.ds(r, n4, stride=NPAIR), :]
                    lo = lax.bitcast_convert_type(u << 16, F32).astype(BF16)
                    hi = lax.bitcast_convert_type(u & jnp.uint32(0xFFFF0000), F32).astype(BF16)
                    dst[(g % 2) * 4 + r, rr, (2 * n) * D:(2 * n + 1) * D] = lo
                    dst[(g % 2) * 4 + r, rr, (2 * n + 1) * D:(2 * n + 2) * D] = hi

    lax.fori_loop(0, 4, lambda t, _: prep(0, t), None)
    for cp in cps2:
        cp.wait()
    tri = lax.broadcasted_iota(jnp.int32, (D, D), 1) <= lax.broadcasted_iota(jnp.int32, (D, D), 0)
    NU = BQ // D

    def pair(j, _):
        for i in range(S // RC):
            rows = slice(i * RC, (i + 1) * RC)
            qs[rows, :] = (_dot(bx[rows, :], wq2[j % 8]) * (D ** -0.5 * LOG2E)).astype(BF16)
            kv = _dot(c[rows, :], wkv[j % 8]).astype(BF16)
            ks[rows, :] = kv[:, 0:2 * D]
            vs[rows, :] = kv[:, 2 * D:4 * D]
        prep((j // 4 + 1) % 4, j % 4)

        def scores(hh, i):
            hs, r0 = slice(hh * D, (hh + 1) * D), i * BQ
            q = qs[r0:r0 + BQ, hs]
            so = _dot_nt(q, ks[0:r0, hs]) if i > 0 else None
            sd = []
            for u in range(NU):
                x = _dot_nt(q[u * D:], ks[r0 + u * D:r0 + (u + 1) * D, hs])
                top = jnp.where(tri, x[:D], NEG)
                sd.append(jnp.concatenate([top, x[D:]], axis=0) if u < NU - 1 else top)
            mm = _reduce(jnp.maximum, [sd[0]] + [so[:, t * D:(t + 1) * D] for t in range(r0 // D)], 1)
            for u in range(1, NU):
                mm = jnp.concatenate([mm[:u * D], jnp.maximum(mm[u * D:], sd[u])], axis=0)
            m = jnp.broadcast_to(jnp.max(mm, axis=1, keepdims=True), (BQ, D))
            return so, sd, m

        sums = []

        def attend(hh, i, so, sd, m):
            hs, r0 = slice(hh * D, (hh + 1) * D), i * BQ
            if len(sums) >= 2:
                lp = sums.pop(0)
                m = jnp.where(lp < 0, lp, m)
            pd = [jnp.exp2(sd[u] - m[u * D:]).astype(BF16) for u in range(NU)]
            pm = pd[0]
            ls = pm.astype(F32)
            if i > 0:
                po = jnp.exp2(so - jnp.concatenate([m] * (r0 // D), axis=1)).astype(BF16)
                ls = _reduce(jnp.add, [ls] + [po[:, t * D:(t + 1) * D].astype(F32) for t in range(r0 // D)], 4)
                pm = jnp.concatenate([po, pm], axis=1)
            o = _dot(pm, vs[0:r0 + D, hs])
            for u in range(1, NU):
                oe = _dot(pd[u], vs[r0 + u * D:r0 + (u + 1) * D, hs])
                o = jnp.concatenate([o[:u * D], o[u * D:] + oe], axis=0)
                ls = jnp.concatenate([ls[:u * D], ls[u * D:] + pd[u].astype(F32)], axis=0)
            sums.append(ls)
            l = jnp.sum(ls, axis=1, keepdims=True)
            ctx[r0:r0 + BQ, hs] = (o * (1.0 / l)).astype(BF16)

        nq = S // BQ
        order = [(0, i) for i in range(nq)] + [(1, i) for i in reversed(range(nq))]
        pend = scores(*order[0])
        for n in range(len(order)):
            nxt = scores(*order[n + 1]) if n + 1 < len(order) else None
            attend(*order[n], *pend)
            pend = nxt
        for t in range(S // RA // NPAIR):
            a_attn(j * (S // RA // NPAIR) + t)
        wo2 = wo[pl.ds(2 * j, 2)].reshape(2 * D, DM)
        for i in range(S // RC):
            rows = slice(i * RC, (i + 1) * RC)
            y = acc[rows, :] + _dot(ctx[rows, :], wo2)
            acc[rows, :] = y
            outb[rows, :] = y.astype(BF16)

    lax.fori_loop(0, NPAIR, pair, None)
    cp_outb = pltpu.make_async_copy(outb, out_h.at[:, DM:2 * DM], sem_ob)
    cp_outb.start()

    def a_out(i, _):
        outa[rows_of(i, RP), :] = _dot(ax[rows_of(i, RP), :], awo[...]).astype(BF16)
        cp_outa(i).start()

    lax.fori_loop(0, S // RP, a_out, None)
    cp_outb.wait()
    for i in range(S // RP):
        cp_outa(i).wait()


@jax.jit
def pallas_concat_heads__sliding_local_dilated__compressed_kv_cla__prompt_kernel(
        A_x, A_wqkv, A_wo, B_x, B_c_kv, B_w_q, B_w_uk, B_w_uv, B_w_o):
    V, DMA = pltpu.VMEM, pltpu.SemaphoreType.DMA
    out = pl.pallas_call(
        _kernel,
        out_shape=jax.ShapeDtypeStruct((S, 2 * DM), BF16),
        in_specs=[pl.BlockSpec(memory_space=pl.ANY)] * 9,
        out_specs=pl.BlockSpec(memory_space=pl.ANY),
        scratch_shapes=[
            V((S, DM), BF16), V((3, DM, DM), BF16), V((DM, DM), BF16),
            V((S, DM), BF16), V((S, DC), BF16),
            V((DM * H, D), BF16), V((DC * H, D), BF16), V((DC * H, D), BF16),
            V((H, D, DM), BF16), V((S, DM), BF16), V((S, DM), BF16),
            V((3, NG, S + PAD, 128), F32), V((NG, DM, 128), F32),
            V((S, 2 * D), BF16), V((S, 2 * D), BF16), V((S, 2 * D), BF16), V((S, 2 * D), BF16),
            V((S, DM), F32), V((8, DM, 2 * D), BF16), V((8, DC, 4 * D), BF16),
            DMA((3,)), DMA((S // RP,)), DMA((7,)), DMA((S // RP,)), DMA,
        ],
        compiler_params=pltpu.CompilerParams(vmem_limit_bytes=110 * 1024 * 1024),
    )(A_x.reshape(S, DM), A_wqkv, A_wo, B_x.reshape(S, DM), B_c_kv.reshape(S, DC),
      B_w_q.reshape(DM * H, D), B_w_uk.reshape(DC * H, D), B_w_uv.reshape(DC * H, D), B_w_o)
    return out.reshape(1, S, 2 * DM)
```

```python
import numpy as np
import jax
import jax.numpy as jnp
from jax import lax
import jax.experimental.pallas as pl
import jax.experimental.pallas.tpu as pltpu

S, DM, DC, H, D = 2048, 640, 512, 32, 128
HA, DA, WIN, DIL = 32, 20, 8, 2
PAD = 16
NG = DM // 128
BQ = 256
RC = 512
RP = 256
RA = 8
NPAIR = H // 2
PLAN = (0, 1, 3, 1, 3, 1, 3, 1, 0, 1, 2, 0)
F32, BF16, U32 = jnp.float32, jnp.bfloat16, jnp.uint32
LOG2E = 1.4426950408889634
NEG = -1e9 * LOG2E
NT = (((1,), (1,)), ((), ()))


def _dot(a, b):
    return jnp.dot(a, b, preferred_element_type=F32)


def _dot_nt(a, b):
    return lax.dot_general(a, b, NT, preferred_element_type=F32)


def _reduce(op, xs, group):
    def tree(ys):
        return ys[0] if len(ys) == 1 else op(tree(ys[:len(ys) // 2]), tree(ys[len(ys) // 2:]))
    r = xs[0]
    for n in range(1, len(xs), group):
        r = op(r, tree(xs[n:n + group]))
    return r


def _kernel(ax_h, wqkv_h, awo_h, bx_h, c_h, wq_h, wuk_h, wuv_h, wo_h, out_h,
            ax, wqkv, awo, bx, c, wq, wuk, wuv, wo, outa, outb,
            qkv, tmp, qs, ks, vs, ctx, acc, wq2, wkv,
            sem_w, sem_x, sem_b, sem_oa, sem_ob, sem_wo):
    def rows_of(i, n):
        return pl.ds(pl.multiple_of(i * n, n), n)

    def cp_wqkv(t):
        return pltpu.make_async_copy(
            wqkv_h.at[:, pl.ds(pl.multiple_of(t * DM, 128), DM)], wqkv.at[t], sem_w.at[t])

    def cp_ax(i):
        return pltpu.make_async_copy(ax_h.at[rows_of(i, RP)], ax.at[rows_of(i, RP)], sem_x.at[i])

    def cp_outa(i):
        return pltpu.make_async_copy(outa.at[rows_of(i, RP)], out_h.at[rows_of(i, RP), 0:DM], sem_oa.at[i])

    def cp_wo(j):
        return pltpu.make_async_copy(wo_h.at[pl.ds(2 * j, 2)], wo.at[pl.ds(2 * j, 2)], sem_wo.at[j])

    def halves(words, n):
        return words.bitcast(BF16).at[0:n]

    first = [(awo_h, awo), (wq_h, halves(wq, DM * H)), (wuk_h, halves(wuk, DC * H)), (wuv_h, halves(wuv, DC * H))]
    second = [(bx_h, bx), (c_h, c)]
    cps = [pltpu.make_async_copy(s, d, sem_b.at[n]) for n, (s, d) in enumerate(first + second)]
    cps1, cps2 = cps[:len(first)], cps[len(first):]
    cp_wqkv(0).start()
    cp_wqkv(1).start()

    qkv[:, :, 0:PAD, :] = jnp.zeros((3, NG, PAD, 128), F32)
    acc[...] = jnp.zeros(acc.shape, F32)

    def permute_rows(w):
        for g in range(NG):
            tmp[g, 0:DM, :] = w[:, g * 128:(g + 1) * 128]
        return jnp.concatenate(
            [jnp.concatenate([tmp[g, pl.ds(d, HA, stride=DA), :] for d in range(DA)], axis=0).astype(BF16)
             for g in range(NG)], axis=1)

    def a_wprep(t, _):
        cp_wqkv(t).wait()

        @pl.when(t == 0)
        def _():
            cp_wqkv(2).start()
            cp_ax(0).start()
            cp_ax(1).start()

        @pl.when(t == 1)
        def _():
            for i in range(2, S // RP):
                cp_ax(i).start()

        @pl.when(t == 2)
        def _():
            for cp in cps1:
                cp.start()

        wqkv[t] = permute_rows(wqkv[t].astype(F32).T)

    lax.fori_loop(0, 3, a_wprep, None)

    def a_proj(i, _):
        @pl.when(i == 1)
        def _():
            for cp in cps2:
                cp.start()

        cp_ax(i).wait()
        for t in range(3):
            y = _dot_nt(ax[rows_of(i, RP), :], wqkv[t])
            if t == 0:
                y = y * (DA ** -0.5 * LOG2E)
            for g in range(NG):
                qkv[t, g, pl.ds(pl.multiple_of(PAD + i * RP, PAD), RP), :] = y[:, g * 128:(g + 1) * 128]

    lax.fori_loop(0, S // RP, a_proj, None)
    for cp in cps1:
        cp.wait()
    awo[...] = permute_rows(awo[...].astype(F32))

    def a_attn(i):
        r0 = pl.multiple_of(i * RA, RA)
        q = qkv[0, :, pl.ds(r0 + PAD, RA), :]
        row = lax.broadcasted_iota(jnp.int32, (RA, 128), 0)
        logits = []
        for w in range(WIN):
            p = q * qkv[1, :, pl.ds(r0 + PAD - DIL * w, RA), :]
            s = p[0] + p[1] + p[2] + p[3] + p[4]
            s = s + pltpu.roll(s, 64, 1)
            s = s + pltpu.roll(s, 32, 1)
            if w > 0:
                s = jnp.where(row >= DIL * w - r0, s, NEG)
            logits.append(s)
        m = _reduce(jnp.maximum, logits, 1)
        es = [jnp.exp2(s - m) for s in logits]
        o = _reduce(jnp.add, [es[w][None] * qkv[2, :, pl.ds(r0 + PAD - DIL * w, RA), :] for w in range(WIN)], 1)
        o = o * pl.reciprocal(_reduce(jnp.add, es, 1), approx=True)[None]
        for g in range(NG):
            ax[pl.ds(r0, RA), g * 128:(g + 1) * 128] = o[g].astype(BF16)
        return o

    def after(o, x):
        o = o[0] + o[1] + o[2] + o[3] + o[4]
        o = jnp.concatenate([o, o], axis=0)
        t = jnp.where(o > np.inf, o, x[0:16, 0:128].astype(F32)).astype(BF16)
        return jnp.concatenate([jnp.concatenate([t, x[0:16, 128:]], axis=1), x[16:]], axis=0)

    def prep(j):
        for dst, w, n in ((wq2, wq, 0), (wkv, wuk, 0), (wkv, wuv, 1)):
            u = w[pl.ds(j, dst.shape[0], stride=NPAIR), :]
            dst[:, (2 * n) * D:(2 * n + 1) * D] = lax.bitcast_convert_type(u << 16, F32).astype(BF16)
            dst[:, (2 * n + 1) * D:(2 * n + 2) * D] = lax.bitcast_convert_type(
                u & jnp.uint32(0xFFFF0000), F32).astype(BF16)

    prep(0)
    cp_wo(0).start()
    for cp in cps2:
        cp.wait()
    for j in range(1, NPAIR):
        cp_wo(j).start()
    tri = lax.broadcasted_iota(jnp.int32, (D, D), 1) <= lax.broadcasted_iota(jnp.int32, (D, D), 0)
    NU = BQ // D

    def pair(j, _):
        plan, done = list(PLAN), [0]

        def side(x):
            for _ in range(plan.pop(0)):
                x = after(a_attn(j * (S // RA // NPAIR) + done[0]), x)
                done[0] += 1
            return x

        cp_wo(j).wait()
        for i in range(S // RC):
            rows = slice(i * RC, (i + 1) * RC)
            qs[rows, :] = (_dot(side(bx[rows, :]), wq2[...]) * (D ** -0.5 * LOG2E)).astype(BF16)
            kv = _dot(side(c[rows, :]), wkv[...]).astype(BF16)
            ks[rows, :] = kv[:, 0:2 * D]
            vs[rows, :] = kv[:, 2 * D:4 * D]

        prep(jnp.minimum(j + 1, NPAIR - 1))

        def scores(hh, i):
            hs, r0 = slice(hh * D, (hh + 1) * D), i * BQ
            q = qs[r0:r0 + BQ, hs]
            so = _dot_nt(q, ks[0:r0, hs]) if i > 0 else None
            sd = []
            for u in range(NU):
                x = _dot_nt(q[u * D:], ks[r0 + u * D:r0 + (u + 1) * D, hs])
                top = jnp.where(tri, x[:D], NEG)
                sd.append(jnp.concatenate([top, x[D:]], axis=0) if u < NU - 1 else top)
            mm = _reduce(jnp.maximum, [sd[0]] + [so[:, t * D:(t + 1) * D] for t in range(r0 // D)], 1)
            for u in range(1, NU):
                mm = jnp.concatenate([mm[:u * D], jnp.maximum(mm[u * D:], sd[u])], axis=0)
            m = jnp.broadcast_to(jnp.max(mm, axis=1, keepdims=True), (BQ, D))
            return so, sd, m

        def attend(hh, i, so, sd, m):
            hs, r0 = slice(hh * D, (hh + 1) * D), i * BQ
            pd = [jnp.exp2(sd[u] - m[u * D:]).astype(BF16) for u in range(NU)]
            pm = pd[0]
            ls = pm.astype(F32)
            if i > 0:
                po = jnp.exp2(so - jnp.concatenate([m] * (r0 // D), axis=1)).astype(BF16)
                ls = _reduce(jnp.add, [ls] + [po[:, t * D:(t + 1) * D].astype(F32) for t in range(r0 // D)], 4)
                pm = jnp.concatenate([po, pm], axis=1)
            o = _dot(pm, vs[0:r0 + D, hs])
            for u in range(1, NU):
                oe = _dot(pd[u], vs[r0 + u * D:r0 + (u + 1) * D, hs])
                o = jnp.concatenate([o[:u * D], o[u * D:] + oe], axis=0)
                ls = jnp.concatenate([ls[:u * D], ls[u * D:] + pd[u].astype(F32)], axis=0)
            l = jnp.sum(ls, axis=1, keepdims=True)
            ctx[r0:r0 + BQ, hs] = (o * pl.reciprocal(l, approx=True)).astype(BF16)

        nq = S // BQ
        order = [(0, i) for i in range(nq)] + [(1, i) for i in reversed(range(nq))]
        pend = scores(*order[0])
        for n in range(len(order)):
            nxt = scores(*order[n + 1]) if n + 1 < len(order) else None
            attend(*order[n], *pend)
            pend = nxt
        wo2 = wo[pl.ds(2 * j, 2)].reshape(2 * D, DM)
        for i in range(S // RC):
            rows = slice(i * RC, (i + 1) * RC)
            y = acc[rows, :] + _dot(side(ctx[rows, :]), wo2)
            acc[rows, :] = y
            outb[rows, :] = y.astype(BF16)

    lax.fori_loop(0, NPAIR, pair, None)
    cp_outb = pltpu.make_async_copy(outb, out_h.at[:, DM:2 * DM], sem_ob)
    cp_outb.start()

    def a_out(i, _):
        outa[rows_of(i, RP), :] = _dot(ax[rows_of(i, RP), :], awo[...]).astype(BF16)
        cp_outa(i).start()

    lax.fori_loop(0, S // RP, a_out, None)
    cp_outb.wait()
    for i in range(S // RP):
        cp_outa(i).wait()


@jax.jit
def pallas_concat_heads__sliding_local_dilated__compressed_kv_cla__prompt_kernel(
        A_x, A_wqkv, A_wo, B_x, B_c_kv, B_w_q, B_w_uk, B_w_uv, B_w_o):
    V, DMA = pltpu.VMEM, pltpu.SemaphoreType.DMA
    out = pl.pallas_call(
        _kernel,
        out_shape=jax.ShapeDtypeStruct((S, 2 * DM), BF16),
        in_specs=[pl.BlockSpec(memory_space=pl.ANY)] * 9,
        out_specs=pl.BlockSpec(memory_space=pl.ANY),
        scratch_shapes=[
            V((S, DM), BF16), V((3, DM, DM), BF16), V((DM, DM), BF16),
            V((S, DM), BF16), V((S, DC), BF16),
            V(((DM + 1) * NPAIR, D), U32), V(((DC + 1) * NPAIR, D), U32),
            V(((DC + 1) * NPAIR, D), U32),
            V((H, D, DM), BF16), V((S, DM), BF16), V((S, DM), BF16),
            V((3, NG, S + PAD, 128), F32), V((NG, DM + 24, 128), F32),
            V((S, 2 * D), BF16), V((S, 2 * D), BF16), V((S, 2 * D), BF16), V((S, 2 * D), BF16),
            V((S, DM), F32), V((DM, 2 * D), BF16), V((DC, 4 * D), BF16),
            DMA((3,)), DMA((S // RP,)), DMA((6,)), DMA((S // RP,)), DMA, DMA((NPAIR,)),
        ],
        compiler_params=pltpu.CompilerParams(vmem_limit_bytes=110 * 1024 * 1024),
    )(A_x.reshape(S, DM), A_wqkv, A_wo, B_x.reshape(S, DM), B_c_kv.reshape(S, DC),
      B_w_q.reshape(DM * H, D), B_w_uk.reshape(DC * H, D), B_w_uv.reshape(DC * H, D), B_w_o)
    return out.reshape(1, S, 2 * DM)
```

```python
import numpy as np
import jax
import jax.numpy as jnp
from jax import lax
import jax.experimental.pallas as pl
import jax.experimental.pallas.tpu as pltpu

S, DM, DC, H, D = 2048, 640, 512, 32, 128
HA, DA, WIN, DIL = 32, 20, 8, 2
PAD = 16
NG = DM // 128
BQ = 256
RC = 512
RP = 256
RA = 8
NPAIR = H // 2
PLAN = (0, 1, 3, 1, 3, 1, 3, 1, 0, 1, 2, 0)
F32, BF16, U32 = jnp.float32, jnp.bfloat16, jnp.uint32
LOG2E = 1.4426950408889634
NEG = -1e9 * LOG2E
NT = (((1,), (1,)), ((), ()))


def _dot(a, b):
    return jnp.dot(a, b, preferred_element_type=F32)


def _dot_nt(a, b):
    return lax.dot_general(a, b, NT, preferred_element_type=F32)


def _reduce(op, xs, group):
    def tree(ys):
        return ys[0] if len(ys) == 1 else op(tree(ys[:len(ys) // 2]), tree(ys[len(ys) // 2:]))
    r = xs[0]
    for n in range(1, len(xs), group):
        r = op(r, tree(xs[n:n + group]))
    return r


def _kernel(ax_h, wqkv_h, awo_h, bx_h, c_h, wq_h, wuk_h, wuv_h, wo_h, out_h,
            ax, wqkv, awo, bx, c, wq, wuk, wuv, wo, outa, outb,
            qkv, tmp, qs, ks, vs, ctx, acc, wq2, wkv,
            sem_w, sem_x, sem_b, sem_oa, sem_ob, sem_wo):
    def rows_of(i, n):
        return pl.ds(pl.multiple_of(i * n, n), n)

    def cp_wqkv(t):
        return pltpu.make_async_copy(
            wqkv_h.at[:, pl.ds(pl.multiple_of(t * DM, 128), DM)], wqkv.at[t], sem_w.at[t])

    def cp_ax(i):
        return pltpu.make_async_copy(ax_h.at[rows_of(i, RP)], ax.at[rows_of(i, RP)], sem_x.at[i])

    def cp_outa(i):
        return pltpu.make_async_copy(outa.at[rows_of(i, RP)], out_h.at[rows_of(i, RP), 0:DM], sem_oa.at[i])

    def cp_wo(j):
        return pltpu.make_async_copy(wo_h.at[pl.ds(2 * j, 2)], wo.at[pl.ds(2 * j, 2)], sem_wo.at[j])

    first = [(awo_h, awo),
             (wq_h.bitcast(U32), wq.at[0:DM * NPAIR]),
             (wuk_h.bitcast(U32), wuk.at[0:DC * NPAIR]),
             (wuv_h.bitcast(U32), wuv.at[0:DC * NPAIR])]
    second = [(bx_h, bx), (c_h, c)]
    cps = [pltpu.make_async_copy(s, d, sem_b.at[n]) for n, (s, d) in enumerate(first + second)]
    cps1, cps2 = cps[:len(first)], cps[len(first):]
    cp_wqkv(0).start()
    cp_wqkv(1).start()

    qkv[:, :, 0:PAD, :] = jnp.zeros((3, NG, PAD, 128), F32)
    acc[...] = jnp.zeros(acc.shape, F32)

    def permute_rows(w):
        for g in range(NG):
            tmp[g, 0:DM, :] = w[:, g * 128:(g + 1) * 128]
        return jnp.concatenate(
            [jnp.concatenate([tmp[g, pl.ds(d, HA, stride=DA), :] for d in range(DA)], axis=0).astype(BF16)
             for g in range(NG)], axis=1)

    def a_wprep(t, _):
        cp_wqkv(t).wait()

        @pl.when(t == 0)
        def _():
            cp_wqkv(2).start()
            cp_ax(0).start()
            cp_ax(1).start()

        @pl.when(t == 1)
        def _():
            for i in range(2, S // RP):
                cp_ax(i).start()

        @pl.when(t == 2)
        def _():
            for cp in cps1:
                cp.start()

        wqkv[t] = permute_rows(wqkv[t].astype(F32).T)

    lax.fori_loop(0, 3, a_wprep, None)

    def a_proj(i, _):
        @pl.when(i == 1)
        def _():
            for cp in cps2:
                cp.start()

        cp_ax(i).wait()
        for t in range(3):
            y = _dot_nt(ax[rows_of(i, RP), :], wqkv[t])
            if t == 0:
                y = y * (DA ** -0.5 * LOG2E)
            for g in range(NG):
                qkv[t, g, pl.ds(pl.multiple_of(PAD + i * RP, PAD), RP), :] = y[:, g * 128:(g + 1) * 128]

    lax.fori_loop(0, S // RP, a_proj, None)
    for cp in cps1:
        cp.wait()
    awo[...] = permute_rows(awo[...].astype(F32))

    def a_attn(i):
        r0 = pl.multiple_of(i * RA, RA)
        q = qkv[0, :, pl.ds(r0 + PAD, RA), :]
        row = lax.broadcasted_iota(jnp.int32, (RA, 128), 0)
        logits = []
        for w in range(WIN):
            p = q * qkv[1, :, pl.ds(r0 + PAD - DIL * w, RA), :]
            s = p[0] + p[1] + p[2] + p[3] + p[4]
            s = s + pltpu.roll(s, 64, 1)
            s = s + pltpu.roll(s, 32, 1)
            if w > 0:
                s = jnp.where(row >= DIL * w - r0, s, NEG)
            logits.append(s)
        m = _reduce(jnp.maximum, logits, 1)
        es = [jnp.exp2(s - m) for s in logits]
        o = _reduce(jnp.add, [es[w][None] * qkv[2, :, pl.ds(r0 + PAD - DIL * w, RA), :] for w in range(WIN)], 1)
        o = o * pl.reciprocal(_reduce(jnp.add, es, 1), approx=True)[None]
        for g in range(NG):
            ax[pl.ds(r0, RA), g * 128:(g + 1) * 128] = o[g].astype(BF16)
        return o

    def after(o, x):
        o = o[0] + o[1] + o[2] + o[3] + o[4]
        o = jnp.concatenate([o, o], axis=0)
        t = jnp.where(o > np.inf, o, x[0:16, 0:128].astype(F32)).astype(BF16)
        return jnp.concatenate([jnp.concatenate([t, x[0:16, 128:]], axis=1), x[16:]], axis=0)

    def prep(j):
        for dst, w, n in ((wq2, wq, 0), (wkv, wuk, 0), (wkv, wuv, 1)):
            u = w[pl.ds(j, dst.shape[0], stride=NPAIR), :]
            dst[:, (2 * n) * D:(2 * n + 1) * D] = lax.bitcast_convert_type(u << 16, F32).astype(BF16)
            dst[:, (2 * n + 1) * D:(2 * n + 2) * D] = lax.bitcast_convert_type(
                u & jnp.uint32(0xFFFF0000), F32).astype(BF16)

    prep(0)
    cp_wo(0).start()
    for cp in cps2:
        cp.wait()
    for j in range(1, NPAIR):
        cp_wo(j).start()
    tri = lax.broadcasted_iota(jnp.int32, (D, D), 1) <= lax.broadcasted_iota(jnp.int32, (D, D), 0)
    NU = BQ // D

    def pair(j, _):
        plan, done = list(PLAN), [0]

        def side(x):
            for _ in range(plan.pop(0)):
                x = after(a_attn(j * (S // RA // NPAIR) + done[0]), x)
                done[0] += 1
            return x

        cp_wo(j).wait()
        for i in range(S // RC):
            rows = slice(i * RC, (i + 1) * RC)
            qs[rows, :] = (_dot(side(bx[rows, :]), wq2[...]) * (D ** -0.5 * LOG2E)).astype(BF16)
            kv = _dot(side(c[rows, :]), wkv[...]).astype(BF16)
            ks[rows, :] = kv[:, 0:2 * D]
            vs[rows, :] = kv[:, 2 * D:4 * D]

        prep(jnp.minimum(j + 1, NPAIR - 1))

        def scores(hh, i):
            hs, r0 = slice(hh * D, (hh + 1) * D), i * BQ
            q = qs[r0:r0 + BQ, hs]
            so = _dot_nt(q, ks[0:r0, hs]) if i > 0 else None
            sd = []
            for u in range(NU):
                x = _dot_nt(q[u * D:], ks[r0 + u * D:r0 + (u + 1) * D, hs])
                top = jnp.where(tri, x[:D], NEG)
                sd.append(jnp.concatenate([top, x[D:]], axis=0) if u < NU - 1 else top)
            mm = _reduce(jnp.maximum, [sd[0]] + [so[:, t * D:(t + 1) * D] for t in range(r0 // D)], 1)
            for u in range(1, NU):
                mm = jnp.concatenate([mm[:u * D], jnp.maximum(mm[u * D:], sd[u])], axis=0)
            m = jnp.broadcast_to(jnp.max(mm, axis=1, keepdims=True), (BQ, D))
            return so, sd, m

        def attend(hh, i, so, sd, m):
            hs, r0 = slice(hh * D, (hh + 1) * D), i * BQ
            pd = [jnp.exp2(sd[u] - m[u * D:]).astype(BF16) for u in range(NU)]
            pm = pd[0]
            ls = pm.astype(F32)
            if i > 0:
                po = jnp.exp2(so - jnp.concatenate([m] * (r0 // D), axis=1)).astype(BF16)
                ls = _reduce(jnp.add, [ls] + [po[:, t * D:(t + 1) * D].astype(F32) for t in range(r0 // D)], 4)
                pm = jnp.concatenate([po, pm], axis=1)
            o = _dot(pm, vs[0:r0 + D, hs])
            for u in range(1, NU):
                oe = _dot(pd[u], vs[r0 + u * D:r0 + (u + 1) * D, hs])
                o = jnp.concatenate([o[:u * D], o[u * D:] + oe], axis=0)
                ls = jnp.concatenate([ls[:u * D], ls[u * D:] + pd[u].astype(F32)], axis=0)
            l = jnp.sum(ls, axis=1, keepdims=True)
            ctx[r0:r0 + BQ, hs] = (o * pl.reciprocal(l, approx=True)).astype(BF16)

        nq = S // BQ
        order = [(0, i) for i in range(nq)] + [(1, i) for i in reversed(range(nq))]
        pend = scores(*order[0])
        for n in range(len(order)):
            nxt = scores(*order[n + 1]) if n + 1 < len(order) else None
            attend(*order[n], *pend)
            pend = nxt
        wo2 = wo[pl.ds(2 * j, 2)].reshape(2 * D, DM)
        for i in range(S // RC):
            rows = slice(i * RC, (i + 1) * RC)
            y = acc[rows, :] + _dot(side(ctx[rows, :]), wo2)
            acc[rows, :] = y
            outb[rows, :] = y.astype(BF16)

    lax.fori_loop(0, NPAIR, pair, None)
    cp_outb = pltpu.make_async_copy(outb, out_h.at[:, DM:2 * DM], sem_ob)
    cp_outb.start()

    def a_out(i, _):
        outa[rows_of(i, RP), :] = _dot(ax[rows_of(i, RP), :], awo[...]).astype(BF16)
        cp_outa(i).start()

    lax.fori_loop(0, S // RP, a_out, None)
    cp_outb.wait()
    for i in range(S // RP):
        cp_outa(i).wait()


@jax.jit
def pallas_concat_heads__sliding_local_dilated__compressed_kv_cla__prompt_kernel(
        A_x, A_wqkv, A_wo, B_x, B_c_kv, B_w_q, B_w_uk, B_w_uv, B_w_o):
    V, DMA = pltpu.VMEM, pltpu.SemaphoreType.DMA
    out = pl.pallas_call(
        _kernel,
        out_shape=jax.ShapeDtypeStruct((S, 2 * DM), BF16),
        in_specs=[pl.BlockSpec(memory_space=pl.ANY)] * 9,
        out_specs=pl.BlockSpec(memory_space=pl.ANY),
        scratch_shapes=[
            V((S, DM), BF16), V((3, DM, DM), BF16), V((DM, DM), BF16),
            V((S, DM), BF16), V((S, DC), BF16),
            V(((DM + 4) * NPAIR, D), U32), V(((DC + 4) * NPAIR, D), U32),
            V(((DC + 4) * NPAIR, D), U32),
            V((H, D, DM), BF16), V((S, DM), BF16), V((S, DM), BF16),
            V((3, NG, S + PAD, 128), F32), V((NG, DM + 24, 128), F32),
            V((S, 2 * D), BF16), V((S, 2 * D), BF16), V((S, 2 * D), BF16), V((S, 2 * D), BF16),
            V((S, DM), F32), V((DM, 2 * D), BF16), V((DC, 4 * D), BF16),
            DMA((3,)), DMA((S // RP,)), DMA((6,)), DMA((S // RP,)), DMA, DMA((NPAIR,)),
        ],
        compiler_params=pltpu.CompilerParams(vmem_limit_bytes=110 * 1024 * 1024),
    )(A_x.reshape(S, DM), A_wqkv, A_wo, B_x.reshape(S, DM), B_c_kv.reshape(S, DC),
      B_w_q.reshape(DM * H, D), B_w_uk.reshape(DC * H, D), B_w_uv.reshape(DC * H, D), B_w_o)
    return out.reshape(1, S, 2 * DM)
```
